```python
import os as _os
_os.environ.setdefault("JAX_PLATFORMS", "cpu")
import jax
import jax.numpy as jnp

def _softmax(x, axis=-1):
    return jax.nn.softmax(x, axis=axis)
def _gelu(x):
    return jax.nn.gelu(x, approximate=True)
def _silu(x):
    return jax.nn.silu(x)
def _sigmoid(x):
    return jax.nn.sigmoid(x)
def _layernorm(x, axis=-1, eps=1e-5):
    m = jnp.mean(x, axis=axis, keepdims=True)
    v = jnp.var(x, axis=axis, keepdims=True)
    return (x - m) / jnp.sqrt(v + eps)
def _scatter_add(tgt, idx, src, axis=0):
    return tgt.at[idx].add(src)
def _segment_sum(src, seg, n):
    return jax.ops.segment_sum(src, seg, n)
class _Rng:
    def __init__(self, key):
        self._k = key
    def _next(self):
        self._k, sub = jax.random.split(self._k)
        return sub
    def normal(self, shape):
        return jax.random.normal(self._next(), shape, dtype=jnp.bfloat16)
    def randint(self, lo, hi, shape):
        return jax.random.randint(self._next(), shape, lo, hi, dtype=jnp.int32)
    def uniform(self, shape, lo=0.0, hi=1.0):
        return jax.random.uniform(self._next(), shape, jnp.bfloat16, lo, hi)
    def permutation(self, n):
        return jax.random.permutation(self._next(), n)


kernel_name = 'standalone__mha_block_cached__near_ridge'

def setup_inputs():
    _rng = _Rng(jax.random.key(int.from_bytes(__import__("os").urandom(4), "little")))
    _w = (lambda a: (lambda t: t.astype(jnp.bfloat16) if jnp.issubdtype(t.dtype, jnp.floating) else t)(jnp.asarray(a)))
    B, Sq, D = 8, 96, 576
    H, Sk, Dh = 32, 96, 128
    return {
        "x": _w((lambda *s: _rng.normal(s) * 0.8)(B, Sq, D)),
        "k_cache": _w((lambda *s: _rng.normal(s) * 0.8)(B, H, Sk, Dh)),
        "v_cache": _w((lambda *s: _rng.normal(s) * 0.05)(B, H, Sk, Dh)),
        "wq": _w((lambda *s: _rng.normal(s) * 0.8)(D, H * Dh) * (D ** -0.5)),
        "wo": _w((lambda *s: _rng.normal(s) * 0.05)(H * Dh, D) * ((H * Dh) ** -0.5)),
    }

def reference(x, k_cache, v_cache, wq, wo):
    B, Sq, D = x.shape
    H, Dh = 32, 128
    q = (lambda x, *d: x.transpose(*d))((x @ wq).reshape(B, Sq, H, Dh), 0, 2, 1, 3)
    scores = jnp.einsum("bhqd,bhkd->bhqk", q, k_cache) * (Dh ** -0.5)
    p = _softmax(scores, axis=-1)
    o = jnp.einsum("bhqk,bhkd->bhqd", p, v_cache)
    return (lambda x, *d: x.transpose(*d))(o, 0, 2, 1, 3).reshape(B, Sq, H * Dh) @ wo
```

```python
import functools
import jax
import jax.numpy as jnp
import jax.experimental.pallas as pl
import jax.experimental.pallas.tpu as pltpu

B, SQ, D = 8, 96, 576
H, SK, DH = 32, 96, 128
M = B * SQ
LOG2E = 1.4426950408889634
C = (DH ** -0.5) * LOG2E
G = 4
NG = H // G
NT = M // 128
DA = 256
XS = 3
NSEM = 4 + (NG - 1) + 1


def slots(g, qs):
    out = []
    for i in range(18):
        sb = i // 2 if i < 16 else None
        pb = i // 2 - 1 if i >= 2 else None
        hs = (0, 1) if i % 2 == 0 else (2, 3)
        s = []
        for h in hs:
            if sb is not None: s.append(('S', g, qs, sb, h))
            if pb is not None: s.append(('P', g, pb, h))
        out.append(s)
    return out


def weave(slot_list, seps):
    out = []
    for i, s in enumerate(slot_list):
        out += s
        if i < len(seps):
            out += seps[i]
    for s in seps[len(slot_list):]:
        out += s
    return out


def kernel(x_hbm, k_hbm, v_hbm, wq_hbm, wot_hbm, out_hbm,
           x_s, k_s, v_s, wq_s, wot_s, q_s, o_s, acc_s, out_s, sems, osem):
    def d_x(b0, b1, sem):
        r = pl.ds(b0 * SQ, (b1 - b0) * SQ)
        return pltpu.make_async_copy(x_hbm.at[r], x_s.at[r], sems.at[sem])
    def d_w(src, dst, g, sem):
        return pltpu.make_async_copy(src.at[:, pl.ds(g * (G * DH), G * DH)], dst.at[g], sems.at[sem])
    def d_kv(src, dst, g, b0, b1, sem):
        return pltpu.make_async_copy(src.at[pl.ds(b0, b1 - b0), pl.ds(g * G, G)],
                                     dst.at[g, pl.ds(b0, b1 - b0)], sems.at[sem])
    def out_desc(j):
        r = pl.ds(j * 128, 128)
        return pltpu.make_async_copy(out_s.at[r], out_hbm.at[r], osem)

    def grp(i):
        if i == 0: return [d_w(wq_hbm, wq_s, 0, 0), d_x(0, XS, 0)]
        if i == 1: return [d_x(XS, B, 1)]
        if i == 2: return [d_w(wq_hbm, wq_s, 1, 2), d_kv(k_hbm, k_s, 0, 0, 4, 2), d_kv(v_hbm, v_s, 0, 0, 4, 2)]
        if i == 3: return [d_kv(k_hbm, k_s, 0, 4, 8, 3), d_kv(v_hbm, v_s, 0, 4, 8, 3), d_w(wot_hbm, wot_s, 0, 3)]
        raise ValueError
    def grp_stage(g):
        s = 3 + g
        return [d_kv(k_hbm, k_s, g, 0, 8, s), d_kv(v_hbm, v_s, g, 0, 8, s),
                d_w(wq_hbm, wq_s, g + 1, s), d_w(wot_hbm, wot_s, g, s)]
    def grp_last():
        g = NG - 1; s = 3 + g
        return [d_kv(k_hbm, k_s, g, 0, 8, s), d_kv(v_hbm, v_s, g, 0, 7, s), d_w(wot_hbm, wot_s, g, s)]
    def grp_fin():
        return [d_kv(v_hbm, v_s, NG - 1, 7, 8, 3 + NG)]

    for i in range(4):
        for d in grp(i): d.start()
    for g in range(1, NG - 1):
        for d in grp_stage(g): d.start()
    for d in grp_last(): d.start()
    for d in grp_fin(): d.start()

    acc_s[:, 512:768] = jnp.zeros((D, 256), jnp.float32)

    pts = {}

    def Q(g, qs, b0, b1):
        r = slice(b0 * SQ, b1 * SQ)
        qq = jnp.dot(x_s[r, :], wq_s[g], preferred_element_type=jnp.float32).astype(jnp.bfloat16)
        for hh in range(G):
            q_s[qs, hh, r, :] = qq[:, hh * DH:(hh + 1) * DH]

    def S(g, qs, b, hh):
        q = q_s[qs, hh, b * SQ:(b + 1) * SQ, :]
        k = k_s[g, b, hh]
        st = jax.lax.dot_general(k, q, (((1,), (1,)), ((), ())), preferred_element_type=jnp.float32)
        m = jnp.max(st, axis=0, keepdims=True)
        pt = jnp.exp2((st - m) * C)
        l = jnp.sum(pt, axis=0, keepdims=True)
        pts[(b, hh)] = (pt * pl.reciprocal(l, approx=True)).astype(jnp.bfloat16)

    def P(g, b, hh):
        v = v_s[g, b, hh]
        o = jax.lax.dot_general(pts.pop((b, hh)), v, (((0,), (0,)), ((), ())), preferred_element_type=jnp.float32)
        o_s[hh, b * SQ:(b + 1) * SQ, :] = o.astype(jnp.bfloat16)

    def T(g, j, part, mode):
        r = {'a': slice(0, DA), 'b': slice(DA, D), 'f': slice(0, D)}[part]
        c = slice(j * 128, (j + 1) * 128)
        o = jnp.concatenate([o_s[hh, c, :] for hh in range(G)], axis=1)
        d = jax.lax.dot_general(wot_s[g, r, :], o, (((1,), (1,)), ((), ())), preferred_element_type=jnp.float32)
        if mode == 'init':
            acc_s[r, c] = d
        elif mode == 'acc':
            acc_s[r, c] += d
        else:
            out_s[c, r] = (acc_s[r, c] + d).T.astype(jnp.bfloat16)

    def run(prog):
        for tok in prog:
            t = tok[0]
            if t == 'W':
                for d in tok[1]: d.wait()
            elif t == 'Q': Q(*tok[1:])
            elif t == 'S': S(*tok[1:])
            elif t == 'P': P(*tok[1:])
            elif t == 'T': T(*tok[1:])
            elif t == 'O': out_desc(tok[1]).start()
            else: raise ValueError(tok)

    def Tp(g, js, mode):
        return [[('T', g, j, p, mode)] for j in js for p in 'ab']
    def Qp(g):
        return [[('Q', g, 0, b, b + 1)] for b in range(B)]

    run([('W', grp(0)), ('Q', 0, 1, 0, XS), ('W', grp(1)), ('Q', 0, 1, XS, B), ('W', grp(2))])
    A = slots(0, 1)
    run(weave(A[:8], Qp(1)))
    run([('W', grp(3))])
    cT = Tp(0, range(4), 'init')
    run(weave(A[8:], [cT[0], cT[1], cT[2], cT[3], cT[4], [], cT[5], [], cT[6], [], cT[7]]))

    def body(g, carry):
        run([('W', grp_stage(g))])
        pT = Tp(g - 1, (4, 5), 'acc'); Qn = Qp(g + 1); cT = Tp(g, range(4), 'acc')
        seps = [pT[0], pT[1], Qn[0], pT[2], Qn[1], pT[3], Qn[2], cT[0], Qn[3], cT[1], Qn[4], cT[2], Qn[5], cT[3],
                Qn[6], cT[4], Qn[7], cT[5], cT[6], cT[7]]
        run(weave(slots(g, 0), seps))
        return carry
    jax.lax.fori_loop(1, NG - 1, body, 0)

    g = NG - 1
    run([('W', grp_last())])
    pT = Tp(g - 1, (4, 5), 'acc'); cT = Tp(g, range(6), 'out')
    A = slots(g, 0)
    seps = [pT[0], [], pT[1], [], pT[2], pT[3], cT[0], cT[1], cT[2], cT[3], cT[4], cT[5], [], [], cT[6], cT[7]]
    run(weave(A[:16], seps))
    run([('O', 0), ('O', 1), ('O', 2), ('O', 3), ('W', grp_fin())])
    run(cT[8] + A[16] + A[17] + cT[9] + [('O', 4)] + cT[10] + cT[11] + [('O', 5)])
    for j in range(NT):
        out_desc(j).wait()


@jax.jit
def pallas_standalone__mha_block_cached__near_ridge_kernel(x, k_cache, v_cache, wq, wo):
    x2 = x.reshape(M, D)
    wot = wo.T
    out = pl.pallas_call(
        kernel,
        in_specs=[pl.BlockSpec(memory_space=pl.ANY)] * 5,
        out_specs=pl.BlockSpec(memory_space=pl.ANY),
        out_shape=jax.ShapeDtypeStruct((M, D), jnp.bfloat16),
        scratch_shapes=[
            pltpu.VMEM((M, D), jnp.bfloat16),
            pltpu.VMEM((NG, B, G, SK, DH), jnp.bfloat16),
            pltpu.VMEM((NG, B, G, SK, DH), jnp.bfloat16),
            pltpu.VMEM((NG, D, G * DH), jnp.bfloat16),
            pltpu.VMEM((NG, D, G * DH), jnp.bfloat16),
            pltpu.VMEM((2, G, M, DH), jnp.bfloat16),
            pltpu.VMEM((G, M, DH), jnp.bfloat16),
            pltpu.VMEM((D, M), jnp.float32),
            pltpu.VMEM((M, D), jnp.bfloat16),
            pltpu.SemaphoreType.DMA((NSEM,)),
            pltpu.SemaphoreType.DMA,
        ],
        compiler_params=pltpu.CompilerParams(vmem_limit_bytes=100 * 1024 * 1024),
    )(x2, k_cache, v_cache, wq, wot)
    return out.reshape(B, SQ, D)
```

```python
import jax
import jax.numpy as jnp
import jax.experimental.pallas as pl
import jax.experimental.pallas.tpu as pltpu

B, SQ, D = 8, 96, 576
H, SK, DH = 32, 96, 128
M = B * SQ
LOG2E = 1.4426950408889634
C = (DH ** -0.5) * LOG2E
G = 4
GW = G * DH
NG = H // G
NT = M // 128
KM = 512
K1 = 128
NR0, NR1 = 1, 5
NSEM = 4

PARTS = {'a': (0, 256), 'b': (256, 576),
         'x': (0, 192), 'y': (192, 384), 'z': (384, 576),
         'p': (0, 256), 'q': (256, 384), 'r': (384, 576)}


def _slots(g, qs):
    out = []
    for i in range(2 * B + 2):
        sb = i // 2 if i < 2 * B else None
        pb = i // 2 - 1 if i >= 2 else None
        s = []
        for h in ((0, 1) if i % 2 == 0 else (2, 3)):
            if sb is not None:
                s.append(('S', g, qs, sb, h))
            if pb is not None:
                s.append(('P', g, pb, h))
        out.append(s)
    return out


def _weave(slot_list, seps):
    out = []
    for i, s in enumerate(slot_list):
        out += s
        if i < len(seps):
            out += seps[i]
    for s in seps[len(slot_list):]:
        out += s
    return out


def _kernel(x_hbm, k_hbm, v_hbm, wq_hbm, wot_hbm, out_hbm,
            x_s, k_s, v_s, wq_s, wqr_s, wot_s, q_s, o_s, acc_s, acc5_s, r_s, out_s, z_s, sems):
    def d_x(k0, k1, sem):
        c = pl.ds(k0, k1 - k0)
        return pltpu.make_async_copy(x_hbm.at[:, c], x_s.at[:, c], sems.at[sem])

    def d_wqr(g0, g1, sem):
        c = pl.ds(g0 * GW, (g1 - g0) * GW)
        return pltpu.make_async_copy(wq_hbm.at[pl.ds(KM, D - KM), c], wqr_s.at[:, c], sems.at[sem])

    def d_wq(g, sem, k0, k1):
        r = pl.ds(k0, k1 - k0)
        return pltpu.make_async_copy(wq_hbm.at[r, pl.ds(g * GW, GW)], wq_s.at[g, r], sems.at[sem])

    def d_wot(g, sem):
        return pltpu.make_async_copy(wot_hbm.at[:, pl.ds(g * GW, GW)], wot_s.at[g], sems.at[sem])

    def d_kv(g, sem):
        return [pltpu.make_async_copy(src.at[:, pl.ds(g * G, G)], dst.at[g], sems.at[sem])
                for src, dst in ((k_hbm, k_s), (v_hbm, v_s))]

    def d_out(r0, n):
        r = pl.ds(r0, n)
        return pltpu.make_async_copy(out_s.at[r], out_hbm.at[r], sems.at[0])

    def gstage(g, s):
        return d_kv(g, s) + [d_wq(g + 1, s, K1, KM), d_wot(g, s)]

    def grp(i):
        if i == 0:
            return [d_wqr(0, NR0, 3), d_x(KM, D, 3)]
        if i == 1:
            return [d_wqr(NR0, NR1, 0)]
        if i == 2:
            return [d_wqr(NR1, NG, 1), d_x(0, K1, 1)] + [d_wq(g, 1, 0, K1) for g in range(NG)]
        return ([d_x(K1, KM, 2), d_wq(0, 2, K1, KM), d_wq(1, 2, K1, KM)] + d_kv(0, 2) + [d_wot(0, 2)])

    def later(i):
        if i < 3:
            s = (i + 3) % 4
            return gstage(1 + 2 * i, s) + gstage(2 + 2 * i, s)
        return d_kv(NG - 1, 2) + [d_wot(NG - 1, 2)]

    for i in range(4):
        for d in grp(i):
            d.start()

    z_s[0] = 0
    pts = {}
    anchors = {}
    outs = []

    def make_anchor(bits):
        w = bits.shape[1]
        acc = None
        for c0 in range(0, w - w % 128, 128):
            for r0 in range(0, bits.shape[0], 8):
                blk = bits[r0:r0 + 8, c0:c0 + 128]
                acc = blk if acc is None else acc | blk
        return acc & z_s[0]

    def inject(val, keys):
        if not keys:
            return val
        a = None
        for kk in keys:
            a = anchors.pop(kk) if a is None else a | anchors.pop(kk)
        bits = pltpu.bitcast(val, jnp.int32)
        top = bits[0:8, :]
        if top.shape[1] > 128:
            top = jnp.concatenate([top[:, 0:128] | a, top[:, 128:]], axis=1)
        else:
            top = top | a
        bits = jnp.concatenate([top, bits[8:, :]], axis=0)
        return pltpu.bitcast(bits, jnp.bfloat16)

    def R(g):
        r_s[g] = jnp.dot(x_s[:, KM:D], wqr_s[:, g * GW:(g + 1) * GW], preferred_element_type=jnp.float32)

    def Q(g, qs, k0, k1, b0, b1, h0=0, h1=G):
        r = slice(b0 * SQ, b1 * SQ)
        n = slice(h0 * DH, h1 * DH)
        d = r_s[g, r, n] + jnp.dot(x_s[r, k0:k1], wq_s[g, k0:k1, n], preferred_element_type=jnp.float32)
        if k1 < KM:
            r_s[g, r, n] = d
        else:
            qq = d.astype(jnp.bfloat16)
            for hh in range(h0, h1):
                q_s[qs, hh, r, :] = qq[:, (hh - h0) * DH:(hh - h0 + 1) * DH]

    def S(g, qs, b, hh, keys=()):
        q = q_s[qs, hh, b * SQ:(b + 1) * SQ, :]
        k = inject(k_s[g, b, hh], keys)
        st = jax.lax.dot_general(k, q, (((1,), (1,)), ((), ())),
                                 preferred_element_type=jnp.float32)
        m = jnp.max(st, axis=0, keepdims=True)
        pt = jnp.exp2((st - m) * C)
        l = jnp.sum(pt, axis=0, keepdims=True)
        pts[(b, hh)] = (pt * (1.0 / l)).astype(jnp.bfloat16)

    def P(g, b, hh):
        o = jax.lax.dot_general(pts.pop((b, hh)), v_s[g, b, hh], (((0,), (0,)), ((), ())),
                                preferred_element_type=jnp.float32)
        o_s[hh, b * SQ:(b + 1) * SQ, :] = o.astype(jnp.bfloat16)

    def T(g, j, part, mode, keys=()):
        r = slice(*PARTS[part])
        c = slice(j * 128, (j + 1) * 128)
        o = jnp.concatenate([o_s[hh, c, :] for hh in range(G)], axis=1)
        d = jax.lax.dot_general(inject(wot_s[g, r, :], keys), o, (((1,), (1,)), ((), ())),
                                preferred_element_type=jnp.float32)
        if mode == 'init':
            acc_s[r, c] = d
        elif mode == 'acc':
            acc_s[r, c] += d
        elif mode == 'acc5':
            t = (acc_s[r, c] + d).T
            acc5_s[:, r] = t
            anchors[('a5', part)] = make_anchor(pltpu.bitcast(t, jnp.int32))
        else:
            t = (acc_s[r, c] + d).T.astype(jnp.bfloat16)
            out_s[c, r] = t
            anchors[(j, part)] = make_anchor(pltpu.bitcast(t, jnp.int32))

    def U(g, r0, r1, n, keys=()):
        n0, n1 = n * 128, min((n + 1) * 128, D)
        c = slice((NT - 1) * 128 + r0, (NT - 1) * 128 + r1)
        o = inject(jnp.concatenate([o_s[hh, c, :] for hh in range(G)], axis=1), keys)
        d = jax.lax.dot_general(o, wot_s[g, n0:n1, :], (((1,), (1,)), ((), ())),
                                preferred_element_type=jnp.float32)
        out_s[c, n0:n1] = (acc5_s[r0:r1, n0:n1] + d).astype(jnp.bfloat16)

    fns = dict(Q=Q, R=R, S=S, P=P, T=T, U=U)

    def run(prog):
        for tok in prog:
            t = tok[0]
            if t == 'W':
                for d in tok[1]:
                    d.wait()
            elif t == 'D':
                for d in tok[1]:
                    d.start()
            elif t == 'O':
                d_out(*tok[1:]).start()
                outs.append(tok[1:])
            else:
                fns[t](*tok[1:])

    def Tp(g, js, mode, parts):
        return [[('T', g, j, p, mode)] for j in js for p in parts]

    def Qh(g):
        return [[('Q', g, 0, K1, KM, b, b + 1, 2 * hf, 2 * hf + 2)] for b in range(B) for hf in range(2)]

    def Qf(g, b):
        return [('Q', g, 0, K1, KM, b, b + 1)]

    def stage(g, first):
        pT = Tp(g - 1, (4, 5), 'acc', 'xyz')
        Qn = Qh(g + 1)
        cT = Tp(g, range(4), 'acc', 'xyz')
        seps = [Qn[i] + pT[i] for i in range(6)]
        seps += [Qn[6 + i] + cT[i] for i in range(8)]
        if first:
            seps += [Qn[14] + cT[8], cT[9], cT[10], cT[11] + Qn[15]]
            run(Qf(g, B - 1))
        else:
            seps += [cT[8], cT[9], cT[10], cT[11]]
        run(_weave(_slots(g, 0), seps))

    run([('W', grp(0))] + [('R', g) for g in range(NR0)] + [('D', later(0))])
    run([('W', grp(1)), ('R', NR0), ('D', later(1))] + [('R', g) for g in range(NR0 + 1, NR1)])
    run([('W', grp(2)), ('R', NR1), ('D', later(2))] + [('R', g) for g in range(NR1 + 1, NG)]
        + [('Q', g, 0, 0, K1, 0, B) for g in range(NG)])
    run([('W', grp(3))])
    K0 = [[('Q', 0, 1, K1, KM, b, b + 1)] for b in range(B)]
    K1h = Qh(1)
    T0 = Tp(0, range(4), 'init', 'ab')
    run(K0[0] + [('D', later(3))] + K0[1])
    acc_s[:, 512:768] = jnp.zeros((D, 256), jnp.float32)
    seps = [K0[2], K1h[0] + K1h[1], K0[3], K1h[2] + K1h[3], K0[4], K1h[4] + K1h[5], K0[5], T0[0], K0[6], T0[1],
            K0[7], T0[2], K1h[6] + K1h[7], T0[3], K1h[8] + K1h[9], T0[4], K1h[10] + K1h[11], T0[5],
            K1h[12] + K1h[13], T0[6], T0[7]]
    run(_weave(_slots(0, 1), seps))

    def body(i, carry):
        g = 1 + 2 * i
        s = (i + 3) % 4
        run([('W', gstage(g, s) + gstage(g + 1, s))])
        stage(g, True)
        stage(g + 1, False)
        return carry

    jax.lax.fori_loop(0, 3, body, 0)

    run([('W', later(3))])
    g = NG - 1
    A = _slots(g, 0)

    def addkeys(slot, keys):
        out = []
        for tok in slot:
            if tok[0] == 'S' and keys:
                out.append(tok + (tuple(keys),))
                keys = None
            else:
                out.append(tok)
        return out

    def t(j, p, keys=()):
        return [('T', g, j, p, 'out', tuple(keys))] + ([('O', j * 128, 128)] if p == 'r' else [])

    for i, keys in ((8, [('a5', 'p')]), (9, [('a5', 'q')]), (10, [(0, 'p'), ('a5', 'r')]), (11, [(0, 'q')]),
                    (12, [(0, 'r')]), (13, [(1, 'p')]), (14, [(1, 'q')]), (15, [(1, 'r')])):
        A[i] = addkeys(A[i], keys)
    seps = Tp(g - 1, (4,), 'acc', 'xyz') + Tp(g - 1, (5,), 'acc5', 'pqr')
    seps[0] = Qf(g, B - 1) + seps[0]
    seps += [t(0, 'p'), t(0, 'q'), t(0, 'r'), t(1, 'p'), t(1, 'q'), t(1, 'r'), t(2, 'p'), t(2, 'q'), t(2, 'r'),
             t(3, 'p'), t(3, 'q', [(2, 'p')]), t(3, 'r', [(2, 'q')]),
             t(4, 'p', [(2, 'r')]), t(4, 'q', [(3, 'p')]), t(4, 'r', [(3, 'q')])]
    run(_weave(A, seps))
    r5 = (NT - 1) * 128
    run([('U', g, 0, 64, 0, ((3, 'r'),)), ('U', g, 0, 64, 1), ('U', g, 0, 64, 2, ((4, 'p'),)), ('U', g, 0, 64, 3),
         ('U', g, 0, 64, 4, ((4, 'q'),)), ('O', r5, 64),
         ('U', g, 64, 128, 0), ('U', g, 64, 128, 1), ('U', g, 64, 128, 2), ('U', g, 64, 128, 3, ((4, 'r'),)),
         ('U', g, 64, 128, 4), ('O', r5 + 64, 64)])
    assert not anchors and not pts
    for a in outs:
        d_out(*a).wait()


@jax.jit
def pallas_standalone__mha_block_cached__near_ridge_kernel(x, k_cache, v_cache, wq, wo):
    out = pl.pallas_call(
        _kernel,
        in_specs=[pl.BlockSpec(memory_space=pl.ANY)] * 5,
        out_specs=pl.BlockSpec(memory_space=pl.ANY),
        out_shape=jax.ShapeDtypeStruct((M, D), jnp.bfloat16),
        scratch_shapes=[
            pltpu.VMEM((M, D), jnp.bfloat16),
            pltpu.VMEM((NG, B, G, SK, DH), jnp.bfloat16),
            pltpu.VMEM((NG, B, G, SK, DH), jnp.bfloat16),
            pltpu.VMEM((NG, KM, GW), jnp.bfloat16),
            pltpu.VMEM((D - KM, H * DH), jnp.bfloat16),
            pltpu.VMEM((NG, D, GW), jnp.bfloat16),
            pltpu.VMEM((2, G, M, DH), jnp.bfloat16),
            pltpu.VMEM((G, M, DH), jnp.bfloat16),
            pltpu.VMEM((D, M), jnp.float32),
            pltpu.VMEM((128, D), jnp.float32),
            pltpu.VMEM((NG, M, GW), jnp.float32),
            pltpu.VMEM((M, D), jnp.bfloat16),
            pltpu.SMEM((1,), jnp.int32),
            pltpu.SemaphoreType.DMA((NSEM,)),
        ],
        compiler_params=pltpu.CompilerParams(vmem_limit_bytes=100 * 1024 * 1024),
    )(x.reshape(M, D), k_cache, v_cache, wq, wo.T)
    return out.reshape(B, SQ, D)
```

```python
import jax
import jax.numpy as jnp
import jax.experimental.pallas as pl
import jax.experimental.pallas.tpu as pltpu

B, SQ, D = 8, 96, 576
H, SK, DH = 32, 96, 128
M = B * SQ
LOG2E = 1.4426950408889634
C = (DH ** -0.5) * LOG2E
G = 4
GW = G * DH
NG = H // G
NT = M // 128
KM = 512
K1 = 128
R0B = 6
NR1 = 5
NSEM = 4

PARTS = {'a': (0, 256), 'b': (256, 576),
         'x': (0, 192), 'y': (192, 384), 'z': (384, 576),
         'p': (0, 256), 'q': (256, 384), 'r': (384, 576)}


def _slots(g, qs):
    out = []
    for i in range(2 * B + 2):
        sb = i // 2 if i < 2 * B else None
        pb = i // 2 - 1 if i >= 2 else None
        s = []
        for h in ((0, 1) if i % 2 == 0 else (2, 3)):
            if sb is not None:
                s.append(('S', g, qs, sb, h))
            if pb is not None:
                s.append(('P', g, pb, h))
        out.append(s)
    return out


def _weave(slot_list, seps):
    out = []
    for i, s in enumerate(slot_list):
        out += s
        if i < len(seps):
            out += seps[i]
    for s in seps[len(slot_list):]:
        out += s
    return out


def _kernel(x_hbm, k_hbm, v_hbm, wq_hbm, wot_hbm, out_hbm,
            x_s, k_s, v_s, wq_s, wqr_s, wqo_s, wot_s, q_s, o_s, acc_s, acc5_s, r_s, out_s, z_s, sems):
    def d_x(k0, k1, sem, b0=0, b1=B):
        c = pl.ds(k0, k1 - k0)
        r = pl.ds(b0 * SQ, (b1 - b0) * SQ)
        return pltpu.make_async_copy(x_hbm.at[r, c], x_s.at[r, c], sems.at[sem])

    def d_wqr(g0, g1, sem):
        c = pl.ds(g0 * GW, (g1 - g0) * GW)
        return pltpu.make_async_copy(wq_hbm.at[pl.ds(KM, D - KM), c], wqr_s.at[:, c], sems.at[sem])

    def d_wq(g, sem, k0, k1):
        r = pl.ds(k0, k1 - k0)
        return pltpu.make_async_copy(wq_hbm.at[r, pl.ds(g * GW, GW)], wq_s.at[g, r], sems.at[sem])

    def d_wot(g, sem):
        return pltpu.make_async_copy(wot_hbm.at[:, pl.ds(g * GW, GW)], wot_s.at[g], sems.at[sem])

    def d_kv(g, sem):
        return [pltpu.make_async_copy(src.at[:, pl.ds(g * G, G)], dst.at[g], sems.at[sem])
                for src, dst in ((k_hbm, k_s), (v_hbm, v_s))]

    def d_out(r0, n):
        r = pl.ds(r0, n)
        return pltpu.make_async_copy(out_s.at[r], out_hbm.at[r], sems.at[0])

    def gstage(g, s):
        return d_kv(g, s) + [d_wq(g + 1, s, K1, KM), d_wot(g, s)]

    def grp(i):
        if i == 0:
            return [d_wqr(0, 1, 0), d_x(KM, D, 0, 0, R0B)]
        if i == 1:
            return [d_x(KM, D, 1, R0B, B), d_wqr(1, NR1, 1)]
        if i == 2:
            return [d_wqr(NR1, NG, 2), d_x(0, K1, 2)] + [d_wq(g, 2, 0, K1) for g in range(NG)]
        return [d_x(K1, KM, 3), d_wq(0, 3, K1, KM), d_wq(1, 3, K1, KM)] + d_kv(0, 3) + [d_wot(0, 3)]

    def later(i):
        if i < 3:
            return gstage(1 + 2 * i, i) + gstage(2 + 2 * i, i)
        return d_kv(NG - 1, 3) + [d_wot(NG - 1, 3)]

    for i in range(4):
        for d in grp(i):
            d.start()

    z_s[0] = 0
    pts = {}
    anchors = {}
    outs = []

    def make_anchor(bits):
        w = bits.shape[1]
        acc = None
        for c0 in range(0, w - w % 128, 128):
            for r0 in range(0, bits.shape[0], 8):
                blk = bits[r0:r0 + 8, c0:c0 + 128]
                acc = blk if acc is None else acc | blk
        return acc & z_s[0]

    def inject(val, keys):
        if not keys:
            return val
        a = None
        for kk in keys:
            a = anchors.pop(kk) if a is None else a | anchors.pop(kk)
        bits = pltpu.bitcast(val, jnp.int32)
        top = bits[0:8, :]
        if top.shape[1] > 128:
            top = jnp.concatenate([top[:, 0:128] | a, top[:, 128:]], axis=1)
        else:
            top = top | a
        bits = jnp.concatenate([top, bits[8:, :]], axis=0)
        return pltpu.bitcast(bits, jnp.bfloat16)

    def R(g, b0=0, b1=B):
        r = slice(b0 * SQ, b1 * SQ)
        r_s[g, r, :] = jnp.dot(x_s[r, KM:D], wqr_s[:, g * GW:(g + 1) * GW], preferred_element_type=jnp.float32)

    def Q(g, qs, k0, k1, b0, b1, h0=0, h1=G, mode='acc', oi=None):
        r = slice(b0 * SQ, b1 * SQ)
        n = slice(h0 * DH, h1 * DH)
        if mode == 'lead':
            s = r_s[g, r, n] + jnp.dot(x_s[r, KM:D], wqo_s[oi], preferred_element_type=jnp.float32)
        elif mode == 'acc':
            s = r_s[g, r, n]
        d = jnp.dot(x_s[r, k0:k1], wq_s[g, k0:k1, n], preferred_element_type=jnp.float32)
        if mode != 'init':
            d = s + d
        if k1 < KM:
            r_s[g, r, n] = d
        else:
            qq = d.astype(jnp.bfloat16)
            for hh in range(h0, h1):
                q_s[qs, hh, r, :] = qq[:, (hh - h0) * DH:(hh - h0 + 1) * DH]

    def S(g, qs, b, hh, keys=()):
        q = q_s[qs, hh, b * SQ:(b + 1) * SQ, :]
        k = inject(k_s[g, b, hh], keys)
        st = jax.lax.dot_general(k, q, (((1,), (1,)), ((), ())),
                                 preferred_element_type=jnp.float32)
        m = jnp.max(st, axis=0, keepdims=True)
        pt = jnp.exp2((st - m) * C)
        l = jnp.sum(pt, axis=0, keepdims=True)
        pts[(b, hh)] = (pt * (1.0 / l)).astype(jnp.bfloat16)

    def P(g, b, hh):
        o = jax.lax.dot_general(pts.pop((b, hh)), v_s[g, b, hh], (((0,), (0,)), ((), ())),
                                preferred_element_type=jnp.float32)
        o_s[hh, b * SQ:(b + 1) * SQ, :] = o.astype(jnp.bfloat16)

    def T(g, j, part, mode, keys=()):
        r = slice(*PARTS[part])
        c = slice(j * 128, (j + 1) * 128)
        o = jnp.concatenate([o_s[hh, c, :] for hh in range(G)], axis=1)
        d = jax.lax.dot_general(inject(wot_s[g, r, :], keys), o, (((1,), (1,)), ((), ())),
                                preferred_element_type=jnp.float32)
        if mode == 'init':
            acc_s[r, c] = d
        elif mode == 'acc':
            acc_s[r, c] += d
        elif mode == 'acc5':
            t = (acc_s[r, c] + d).T
            acc5_s[:, r] = t
            anchors[('a5', part)] = make_anchor(pltpu.bitcast(t, jnp.int32))
        else:
            t = (acc_s[r, c] + d).T.astype(jnp.bfloat16)
            out_s[c, r] = t
            anchors[(j, part)] = make_anchor(pltpu.bitcast(t, jnp.int32))

    def U(g, r0, r1, n, keys=()):
        n0, n1 = n * 128, min((n + 1) * 128, D)
        c = slice((NT - 1) * 128 + r0, (NT - 1) * 128 + r1)
        o = inject(jnp.concatenate([o_s[hh, c, :] for hh in range(G)], axis=1), keys)
        d = jax.lax.dot_general(o, wot_s[g, n0:n1, :], (((1,), (1,)), ((), ())),
                                preferred_element_type=jnp.float32)
        out_s[c, n0:n1] = (acc5_s[r0:r1, n0:n1] + d).astype(jnp.bfloat16)

    fns = dict(Q=Q, R=R, S=S, P=P, T=T, U=U)

    def run(prog):
        for tok in prog:
            t = tok[0]
            if t == 'W':
                for d in tok[1]:
                    d.wait()
            elif t == 'D':
                for d in tok[1]:
                    d.start()
            elif t == 'O':
                d_out(*tok[1:]).start()
                outs.append(tok[1:])
            else:
                fns[t](*tok[1:])

    def Tp(g, js, mode, parts):
        return [[('T', g, j, p, mode)] for j in js for p in parts]

    def Qh(g):
        return [[('Q', g, 0, K1, KM, b, b + 1, 2 * hf, 2 * hf + 2)] for b in range(B) for hf in range(2)]

    def Qf(g, b, i):
        return [('Q', g, 0, K1, KM, b, b + 1, 0, G, 'lead', i)]

    def stage(g, first, oi=None):
        pT = Tp(g - 1, (4, 5), 'acc', 'xyz')
        Qn = Qh(g + 1)
        cT = Tp(g, range(4), 'acc', 'xyz')
        seps = [Qn[i] + pT[i] for i in range(6)]
        seps += [Qn[6 + i] + cT[i] for i in range(8)]
        if first:
            seps += [Qn[14] + cT[8], cT[9], cT[10], cT[11] + Qn[15]]
            run(Qf(g, B - 1, oi))
        else:
            seps += [cT[8], cT[9], cT[10], cT[11]]
        run(_weave(_slots(g, 0), seps))

    def Rg(g):
        return ('R', g, 0, B - 1) if (g % 2 or g == 6) else ('R', g)

    def T0g(g):
        if g % 2:
            return [('Q', g, 0, 0, K1, 0, B - 1), ('Q', g, 0, 0, K1, B - 1, B, 0, G, 'init')]
        return [('Q', g, 0, 0, K1, 0, B - 1 if g == 6 else B)]

    order = [g for g in range(NG) if g != 6] + [6]
    run([('W', grp(0)), ('R', 0, 0, R0B), ('D', later(0))])
    run([('W', grp(1)), ('R', 0, R0B, B), ('D', later(1))] + [Rg(g) for g in range(1, NR1)])
    run([('W', grp(2)), Rg(NR1), ('D', later(2))] + [Rg(g) for g in order if g > NR1]
        + sum([T0g(g) for g in order], []))
    for i in range(NG // 2):
        wqo_s[i] = wqr_s[:, (2 * i + 1) * GW:(2 * i + 2) * GW]
    run([('W', grp(3)), ('R', 6, B - 1, B), ('Q', 6, 0, 0, K1, B - 1, B)])
    K0 = [[('Q', 0, 1, K1, KM, b, b + 1)] for b in range(B)]
    K1h = Qh(1)
    T0 = Tp(0, range(4), 'init', 'ab')
    run(K0[0] + [('D', later(3))] + K0[1])
    acc_s[:, 512:768] = jnp.zeros((D, 256), jnp.float32)
    seps = [K0[2], K1h[0] + K1h[1], K0[3], K1h[2] + K1h[3], K0[4], K1h[4] + K1h[5], K0[5], T0[0], K0[6], T0[1],
            K0[7], T0[2], K1h[6] + K1h[7], T0[3], K1h[8] + K1h[9], T0[4], K1h[10] + K1h[11], T0[5],
            K1h[12] + K1h[13], T0[6], T0[7]]
    run(_weave(_slots(0, 1), seps))

    def body(i, carry):
        g = 1 + 2 * i
        run([('W', gstage(g, i) + gstage(g + 1, i))])
        stage(g, True, i)
        stage(g + 1, False)
        return carry

    jax.lax.fori_loop(0, 3, body, 0)

    run([('W', later(3))])
    g = NG - 1
    A = _slots(g, 0)

    def addkeys(slot, keys):
        out = []
        for tok in slot:
            if tok[0] == 'S' and keys:
                out.append(tok + (tuple(keys),))
                keys = None
            else:
                out.append(tok)
        return out

    def t(j, p, keys=()):
        return [('T', g, j, p, 'out', tuple(keys))] + ([('O', j * 128, 128)] if p == 'r' else [])

    for i, keys in ((8, [('a5', 'p')]), (9, [('a5', 'q')]), (10, [(0, 'p'), ('a5', 'r')]), (11, [(0, 'q')]),
                    (12, [(0, 'r')]), (13, [(1, 'p')]), (14, [(1, 'q')]), (15, [(1, 'r')])):
        A[i] = addkeys(A[i], keys)
    seps = Tp(g - 1, (4,), 'acc', 'xyz') + Tp(g - 1, (5,), 'acc5', 'pqr')
    run(Qf(g, B - 1, NG // 2 - 1))
    seps += [t(0, 'p'), t(0, 'q'), t(0, 'r'), t(1, 'p'), t(1, 'q'), t(1, 'r'), t(2, 'p'), t(2, 'q'), t(2, 'r'),
             t(3, 'p'), t(3, 'q', [(2, 'p')]), t(3, 'r', [(2, 'q')]),
             t(4, 'p', [(2, 'r')]), t(4, 'q', [(3, 'p')]), t(4, 'r', [(3, 'q')])]
    run(_weave(A, seps))
    r5 = (NT - 1) * 128
    run([('U', g, 0, 64, 0, ((3, 'r'),)), ('U', g, 0, 64, 1), ('U', g, 0, 64, 2, ((4, 'p'),)), ('U', g, 0, 64, 3),
         ('U', g, 0, 64, 4, ((4, 'q'),)), ('O', r5, 64),
         ('U', g, 64, 128, 0), ('U', g, 64, 128, 1), ('U', g, 64, 128, 2), ('U', g, 64, 128, 3, ((4, 'r'),)),
         ('U', g, 64, 128, 4), ('O', r5 + 64, 64)])
    assert not anchors and not pts
    for a in outs:
        d_out(*a).wait()


@jax.jit
def pallas_standalone__mha_block_cached__near_ridge_kernel(x, k_cache, v_cache, wq, wo):
    out = pl.pallas_call(
        _kernel,
        in_specs=[pl.BlockSpec(memory_space=pl.ANY)] * 5,
        out_specs=pl.BlockSpec(memory_space=pl.ANY),
        out_shape=jax.ShapeDtypeStruct((M, D), jnp.bfloat16),
        scratch_shapes=[
            pltpu.VMEM((M, D), jnp.bfloat16),
            pltpu.VMEM((NG, B, G, SK, DH), jnp.bfloat16),
            pltpu.VMEM((NG, B, G, SK, DH), jnp.bfloat16),
            pltpu.VMEM((NG, KM, GW), jnp.bfloat16),
            pltpu.VMEM((D - KM, H * DH), jnp.bfloat16),
            pltpu.VMEM((NG // 2, D - KM, GW), jnp.bfloat16),
            pltpu.VMEM((NG, D, GW), jnp.bfloat16),
            pltpu.VMEM((2, G, M, DH), jnp.bfloat16),
            pltpu.VMEM((G, M, DH), jnp.bfloat16),
            pltpu.VMEM((D, M), jnp.float32),
            pltpu.VMEM((128, D), jnp.float32),
            pltpu.VMEM((NG, M, GW), jnp.float32),
            pltpu.VMEM((M, D), jnp.bfloat16),
            pltpu.SMEM((1,), jnp.int32),
            pltpu.SemaphoreType.DMA((NSEM,)),
        ],
        compiler_params=pltpu.CompilerParams(vmem_limit_bytes=100 * 1024 * 1024),
    )(x.reshape(M, D), k_cache, v_cache, wq, wo.T)
    return out.reshape(B, SQ, D)
```
